```python
import os as _os
_os.environ.setdefault("JAX_PLATFORMS", "cpu")
import jax
import jax.numpy as jnp

def _softmax(x, axis=-1):
    return jax.nn.softmax(x, axis=axis)
def _gelu(x):
    return jax.nn.gelu(x, approximate=True)
def _silu(x):
    return jax.nn.silu(x)
def _sigmoid(x):
    return jax.nn.sigmoid(x)
def _layernorm(x, axis=-1, eps=1e-5):
    m = jnp.mean(x, axis=axis, keepdims=True)
    v = jnp.var(x, axis=axis, keepdims=True)
    return (x - m) / jnp.sqrt(v + eps)
def _scatter_add(tgt, idx, src, axis=0):
    return tgt.at[idx].add(src)
def _segment_sum(src, seg, n):
    return jax.ops.segment_sum(src, seg, n)
class _Rng:
    def __init__(self, key):
        self._k = key
    def _next(self):
        self._k, sub = jax.random.split(self._k)
        return sub
    def normal(self, shape):
        return jax.random.normal(self._next(), shape, dtype=jnp.bfloat16)
    def randint(self, lo, hi, shape):
        return jax.random.randint(self._next(), shape, lo, hi, dtype=jnp.int32)
    def uniform(self, shape, lo=0.0, hi=1.0):
        return jax.random.uniform(self._next(), shape, jnp.bfloat16, lo, hi)
    def permutation(self, n):
        return jax.random.permutation(self._next(), n)


kernel_name = 'parallel_sum__grouped_kv_mqa__dense_activation_silu__prompt'

def setup_inputs():
    _rng = _Rng(jax.random.key(int.from_bytes(__import__("os").urandom(4), "little")))
    _w = (lambda a: (lambda t: t.astype(jnp.bfloat16) if jnp.issubdtype(t.dtype, jnp.floating) else t)(jnp.asarray(a)))
    def _A_setup():
        B, S, D, H = 1, 2048, 512, 32
        Dh = D // H
        return {
            "x": _w((lambda *s: _rng.normal(s) * 0.05)(B, S, D)),
            "wq": _w((lambda *s: _rng.normal(s) * 0.05)(D, H * Dh)),
            "wk": _w((lambda *s: _rng.normal(s) * 0.05)(D, Dh)),
            "wv": _w((lambda *s: _rng.normal(s) * 0.05)(D, Dh)),
            "wo": _w((lambda *s: _rng.normal(s) * 0.05)(H * Dh, D)),
        }
    _A_in = _A_setup()

    def _B_setup():
        B, S, D, F = 1, 2048, 512, 1376
        return {
            "x": _w((lambda *s: _rng.normal(s) * 0.05)(B, S, D)),
            "w1": _w((lambda *s: _rng.normal(s) * 0.05)(D, F) * (D ** -0.5)),
            "w2": _w((lambda *s: _rng.normal(s) * 0.05)(F, D) * (F ** -0.5)),
        }
    _B_in = _B_setup()

    return {
        "A_x": _A_in["x"],
        "A_wq": _A_in["wq"],
        "A_wk": _A_in["wk"],
        "A_wv": _A_in["wv"],
        "A_wo": _A_in["wo"],
        "B_x": _B_in["x"],
        "B_w1": _B_in["w1"],
        "B_w2": _B_in["w2"],
    }

def reference(A_x, A_wq, A_wk, A_wv, A_wo, B_x, B_w1, B_w2):
    def _A_ref(x, wq, wk, wv, wo):
        B, S, D = x.shape
        H = 32
        Dh = D // H
        q = (lambda x, *d: x.transpose(*d))((x @ wq).reshape(B, S, H, Dh), 0, 2, 1, 3)
        k = x @ wk
        v = x @ wv
        scores = jnp.einsum("bhqd,bkd->bhqk", q, k) * (Dh ** -0.5)
        p = _softmax(scores, axis=-1)
        o = jnp.einsum("bhqk,bkd->bhqd", p, v)
        return (lambda x, *d: x.transpose(*d))(o, 0, 2, 1, 3).reshape(B, S, H * Dh) @ wo

    def _B_ref(x, w1, w2):
        h = jnp.einsum("bsd,df->bsf", x, w1)
        h = _silu(h)
        out = jnp.einsum("bsf,fd->bsd", h, w2)
        return out

    x = A_x
    xn = _layernorm(x, axis=-1)
    return x + _A_ref(xn, A_wq, A_wk, A_wv, A_wo) + _B_ref(xn, B_w1, B_w2)
```

```python
import functools
import math

import jax
import jax.numpy as jnp
import jax.experimental.pallas as pl
import jax.experimental.pallas.tpu as pltpu

_H = 32
_EPS = 1e-5
_BQ = 1024
_CK = 128


def _kernel(x_ref, wq_ref, wk_ref, wv_ref, wo_ref, w1_ref, w2_ref, o_ref,
            xn_ref, k_ref, vt_ref, qt_ref, ot_ref, s0_ref, s1_ref, *, bq):
    step = pl.program_id(0)
    seq, d = x_ref.shape
    dh = d // _H
    f32, bf16 = jnp.float32, jnp.bfloat16
    nt = (((1,), (1,)), ((), ()))

    @pl.when(step == 0)
    def _():
        def ln(i, c):
            rows = pl.ds(pl.multiple_of(i * bq, bq), bq)
            x = x_ref[rows, :].astype(f32)
            xc = x - jnp.mean(x, axis=-1, keepdims=True)
            var = jnp.mean(xc * xc, axis=-1, keepdims=True)
            xn = (xc * jax.lax.rsqrt(var + _EPS)).astype(bf16)
            xn_ref[rows, :] = xn
            k_ref[rows, :] = jax.lax.dot_general(xn, wk_ref[...], nt, preferred_element_type=f32).astype(bf16)
            return c

        jax.lax.fori_loop(0, seq // bq, ln, 0)
        vt = jax.lax.dot_general(wv_ref[...], xn_ref[...], nt,
                                 preferred_element_type=f32)
        vt_ref[0:dh, :] = vt.astype(bf16)
        vt_ref[dh:2 * dh, :] = jnp.ones((dh, seq), bf16)

    rows = pl.ds(pl.multiple_of(step * bq, bq), bq)
    xn = xn_ref[rows, :]
    q = jnp.dot(xn, wq_ref[...], preferred_element_type=f32)
    qt_ref[...] = (q * (dh ** -0.5 * math.log2(math.e))).T.astype(bf16)

    def head(h):
        return pl.ds(pl.multiple_of(h * dh, dh), dh)

    def stage(hs, ss, ha, sa, m):
        mx = o = None
        for c in range(seq // _CK):
            keys = slice(c * _CK, (c + 1) * _CK)
            if ss is not None:
                s = jnp.dot(k_ref[keys, :], qt_ref[head(hs), :], preferred_element_type=f32)
                ss[keys, :] = s
                s = jnp.max(s.reshape(_CK // 8, 8, bq), axis=0)
                mx = s if mx is None else jnp.maximum(mx, s)
            if sa is not None:
                p = jnp.exp2(sa[keys, :] - m).astype(bf16)
                pv = jnp.dot(vt_ref[:, keys], p, preferred_element_type=f32)
                o = pv if o is None else o + pv
        if sa is not None:
            ot_ref[head(ha), :] = o[0:dh] / o[dh:2 * dh]
        if ss is not None:
            return jnp.max(mx, axis=0, keepdims=True)

    def pair(i, m):
        m = stage(2 * i + 1, s1_ref, 2 * i, s0_ref, m)
        return stage(2 * i + 2, s0_ref, 2 * i + 1, s1_ref, m)

    m = jax.lax.fori_loop(0, _H // 2 - 1, pair, stage(0, s0_ref, None, None, None))
    m = stage(_H - 1, s1_ref, _H - 2, s0_ref, m)
    stage(None, None, _H - 1, s1_ref, m)

    attn = jnp.dot(ot_ref[...].T.astype(bf16), wo_ref[...], preferred_element_type=f32)
    hid = jax.lax.dot_general(xn, w1_ref[...], nt, preferred_element_type=f32)
    hid = (hid * jax.nn.sigmoid(hid)).astype(bf16)
    ffn = jnp.dot(hid, w2_ref[...], preferred_element_type=f32)
    o_ref[...] = (x_ref[rows, :].astype(f32) + attn + ffn).astype(o_ref.dtype)


@jax.jit
def pallas_parallel_sum__grouped_kv_mqa__dense_activation_silu__prompt_kernel(
    A_x: jax.Array,
    A_wq: jax.Array,
    A_wk: jax.Array,
    A_wv: jax.Array,
    A_wo: jax.Array,
    B_x: jax.Array,
    B_w1: jax.Array,
    B_w2: jax.Array,
):
    del B_x
    b, seq, d = A_x.shape
    assert b == 1 and seq % _BQ == 0
    dh = d // _H
    bq = _BQ
    full = lambda a: pl.BlockSpec(a.shape, lambda i: (0,) * a.ndim)
    x2 = A_x.reshape(seq, d)
    args = (x2, A_wq, A_wk.T, A_wv.T, A_wo, B_w1.T, B_w2)
    out = pl.pallas_call(
        functools.partial(_kernel, bq=bq),
        grid=(seq // bq,),
        in_specs=[full(a) for a in args],
        out_specs=pl.BlockSpec((bq, d), lambda i: (i, 0)),
        out_shape=jax.ShapeDtypeStruct((seq, d), A_x.dtype),
        scratch_shapes=[
            pltpu.VMEM((seq, d), jnp.bfloat16),
            pltpu.VMEM((seq, dh), jnp.bfloat16),
            pltpu.VMEM((2 * dh, seq), jnp.bfloat16),
            pltpu.VMEM((d, bq), jnp.bfloat16),
            pltpu.VMEM((d, bq), jnp.float32),
            pltpu.VMEM((seq, bq), jnp.float32),
            pltpu.VMEM((seq, bq), jnp.float32),
        ],
        compiler_params=pltpu.CompilerParams(
            dimension_semantics=("arbitrary",), vmem_limit_bytes=100 * 2**20),
    )(*args)
    return out.reshape(b, seq, d)
```
